```python
import jax
import jax.numpy as jnp

def _softmax(x, axis=-1):
    return jax.nn.softmax(x, axis=axis)

def _gelu(x):
    return jax.nn.gelu(x, approximate=True)

def _silu(x):
    return jax.nn.silu(x)

def _sigmoid(x):
    return jax.nn.sigmoid(x)

def _layernorm(x, axis=-1, eps=1e-05):
    m = jnp.mean(x, axis=axis, keepdims=True)
    v = jnp.var(x, axis=axis, keepdims=True)
    return (x - m) / jnp.sqrt(v + eps)

def _scatter_add(tgt, idx, src, axis=0):
    return tgt.at[idx].add(src)

def _segment_sum(src, seg, n):
    return jax.ops.segment_sum(src, seg, n)

class _Rng:

    def __init__(self, key):
        self._k = key

    def _next(self):
        self._k, sub = jax.random.split(self._k)
        return sub

    def normal(self, shape):
        return jax.random.normal(self._next(), shape, dtype=jnp.bfloat16)

    def randint(self, lo, hi, shape):
        return jax.random.randint(self._next(), shape, lo, hi, dtype=jnp.int32)

    def uniform(self, shape, lo=0.0, hi=1.0):
        return jax.random.uniform(self._next(), shape, jnp.bfloat16, lo, hi)

    def permutation(self, n):
        return jax.random.permutation(self._next(), n)
kernel_name = 'sequential_preLN__memory_aug_recurrent_mem_tr__moe_arch_mod__prompt'

def setup_inputs():
    _rng = _Rng(jax.random.key(int.from_bytes(__import__("os").urandom(4), "little")))
    _w = lambda a: (lambda t: t.astype(jnp.bfloat16) if jnp.issubdtype(t.dtype, jnp.floating) else t)(jnp.asarray(a))

    def _A_setup():
        B, S, Dm = (1, 2048, 512)
        H, Dh = (32, 128)
        M, seg = (8, 32)
        seg = min(seg, S)
        S = S // seg * seg
        return {'x': _w((lambda *s: _rng.normal(s) * 0.05)(B, S, Dm)), 'mem0': _w((lambda *s: _rng.normal(s) * 0.05)(B, M, Dm)), 'Wq': _w((lambda *s: _rng.normal(s) * 0.05)(Dm, H, Dh) * Dm ** (-0.5)), 'Wk': _w((lambda *s: _rng.normal(s) * 0.05)(Dm, H, Dh) * Dm ** (-0.5)), 'Wv': _w((lambda *s: _rng.normal(s) * 0.05)(Dm, H, Dh) * Dm ** (-0.5)), 'Wo': _w((lambda *s: _rng.normal(s) * 0.05)(H, Dh, Dm) * (H * Dh) ** (-0.5)), 'seg_len': seg}
    _A_in = _A_setup()

    def _B_setup():
        B, S, D, F, C = (1, 2048, 512, 1792, 2)
        return {'x': _w((lambda *s: _rng.normal(s) * 0.05)(B, S, D)), 'w_r': _w((lambda *s: _rng.normal(s) * 0.05)(D)), 'w_gate': _w((lambda *s: _rng.normal(s) * 0.05)(D, F)), 'w_up': _w((lambda *s: _rng.normal(s) * 0.05)(D, F)), 'w_down': _w((lambda *s: _rng.normal(s) * 0.05)(F, D))}
    _B_in = _B_setup()
    return {'A_x': _A_in['x'], 'A_mem0': _A_in['mem0'], 'A_Wq': _A_in['Wq'], 'A_Wk': _A_in['Wk'], 'A_Wv': _A_in['Wv'], 'A_Wo': _A_in['Wo'], 'A_seg_len': _A_in['seg_len'], 'B_x': _B_in['x'], 'B_w_r': _B_in['w_r'], 'B_w_gate': _B_in['w_gate'], 'B_w_up': _B_in['w_up'], 'B_w_down': _B_in['w_down']}

def reference(A_x, A_mem0, A_Wq, A_Wk, A_Wv, A_Wo, A_seg_len, B_x, B_w_r, B_w_gate, B_w_up, B_w_down):

    def _A_ref(x, mem0, Wq, Wk, Wv, Wo, seg_len):
        B, S, Dm = x.shape
        H, Dh = (Wq.shape[1], Wq.shape[2])
        M = mem0.shape[1]
        scale = Dh ** (-0.5)
        n_seg = S // seg_len
        L = M + seg_len
        idx = jnp.arange(L)
        mask = (idx[:, None] < M) | (idx[:, None] >= idx[None, :])
        mem = mem0
        outs = []
        for s in range(n_seg):
            xs = x[:, s * seg_len:(s + 1) * seg_len, :].copy()
            h = jnp.concatenate([mem, xs], axis=1)
            q = jnp.einsum('btd,dhe->bhte', h, Wq)
            k = jnp.einsum('btd,dhe->bhte', h, Wk)
            v = jnp.einsum('btd,dhe->bhte', h, Wv)
            scores = jnp.einsum('bhqe,bhke->bhqk', q, k) * scale
            scores = jnp.where(mask[None, None], scores, -1000000000.0)
            p = _softmax(scores, axis=-1)
            o = jnp.einsum('bhqk,bhke->bhqe', p, v)
            o = jnp.einsum('bhte,hed->btd', o, Wo)
            mem = o[:, :M, :].copy()
            outs.append(o[:, M:, :])
        return jnp.concatenate(outs, axis=1)

    def _B_ref(x, w_r, w_gate, w_up, w_down):
        B, S, D = x.shape
        C = 2
        r = x @ w_r
        idx = jnp.argsort(-r, axis=-1)[:, :C]
        idx_e = jnp.repeat(idx.reshape(B, C, 1), D, axis=2)
        x_sel = jnp.take_along_axis(x, idx_e, axis=1)
        g = _silu(x_sel @ w_gate)
        u = x_sel @ w_up
        y = g * u @ w_down
        r_sel = _sigmoid(jnp.take_along_axis(r, idx, axis=1))
        y = y * r_sel.reshape(B, C, 1)
        b_off = (jnp.arange(B) * S).reshape(B, 1)
        flat_idx = (idx + b_off).reshape(B * C)
        zero = (x * 0.0).reshape(B * S, D)
        upd = _scatter_add(zero, flat_idx, y.reshape(B * C, D), axis=0)
        return x + upd.reshape(B, S, D)
    x = A_x
    h = x + _A_ref(_layernorm(x, axis=-1), A_mem0, A_Wq, A_Wk, A_Wv, A_Wo, A_seg_len)
    h2 = h + _B_ref(_layernorm(h, axis=-1), B_w_r, B_w_gate, B_w_up, B_w_down)
    return h2
```

```python
import functools

import jax
import jax.numpy as jnp
import numpy as np
from jax import lax
from jax.experimental import pallas as pl
from jax.experimental.pallas import tpu as pltpu

F32 = jnp.float32
BF16 = jnp.bfloat16
U32 = jnp.uint32

_EPS = float(np.asarray(1e-5, dtype=BF16))
_LOG2E = float(np.log2(np.e))
_MASKED = -1000000000.0
_NT = (((1,), (1,)), ((), ()))
_TOPC = 2


def _rnd(a):
    return a.astype(BF16).astype(F32)


def _layernorm(a):
    n = a.shape[-1]
    mean = jnp.sum(a, axis=-1, keepdims=True) * (1.0 / n)
    cen = a - mean
    var = jnp.sum(cen * cen, axis=-1, keepdims=True) * (1.0 / n)
    std = _rnd(jnp.sqrt(_rnd(_rnd(var) + _EPS)))
    return _rnd(_rnd(a - _rnd(mean)) * (1.0 / std))


def _dot(a, b):
    return jnp.dot(a, b, preferred_element_type=F32)


def _dot_nt(a, b):
    return lax.dot_general(a, b, _NT, preferred_element_type=F32)


def _softmax_terms(scores, mask, fill, scale):
    s = jnp.where(mask, scores * scale, fill)
    e = jnp.exp2((s - jnp.max(s, axis=-1, keepdims=True)) * _LOG2E)
    return e.astype(BF16), 1.0 / jnp.sum(e, axis=-1, keepdims=True)


def _kernel(x_hbm, mem0_ref, wq_hbm, wk_hbm, wv_hbm, wo_hbm, wr_ref, wg_hbm, wu_hbm, wd_hbm,
            out_hbm,
            x_v, stage, wo_raw, wg_v, wu_v, wd_v, wqkv, wo, xn, pre, att, r_v, out_v, sems,
            *, nseg, seg, nmem, nheads, dh, dm):
    scale = float(np.asarray(dh ** -0.5, dtype=BF16))
    npre = nmem
    rows_pre = nseg * npre
    hc = 16
    nchunk = nheads // hc

    x_cp = pltpu.make_async_copy(x_hbm, x_v, sems.at[0])
    x_cp.start()
    w_cps = []
    for m, w_hbm in enumerate((wq_hbm, wk_hbm, wv_hbm)):
        w32 = w_hbm.bitcast(U32)
        for c in range(nchunk):
            i = m * nchunk + c
            cp = pltpu.make_async_copy(
                w32.at[:, pl.ds(c * hc // 2, hc // 2), :], stage.at[i], sems.at[1 + i])
            cp.start()
            w_cps.append(cp)
    base = 1 + 3 * nchunk
    wo_cp = pltpu.make_async_copy(wo_hbm, wo_raw, sems.at[base])
    wo_cp.start()
    ffn_cps = [pltpu.make_async_copy(src, dst, sems.at[base + 1 + i])
               for i, (src, dst) in enumerate(((wg_hbm, wg_v), (wu_hbm, wu_v), (wd_hbm, wd_v)))]
    for cp in ffn_cps:
        cp.start()

    x_cp.wait()

    def ln1(g, carry):
        a = x_v[pl.ds(g * 8, 8)].astype(F32).reshape(8 * seg, dm)
        xn[pl.ds(g * 8, 8)] = _layernorm(a).reshape(8, seg, dm)
        return carry

    lax.fori_loop(0, nseg // 8, ln1, 0)

    stage2d = stage.reshape(3 * nchunk * dm * hc // 2, dh)

    def prologue(i, carry):
        pltpu.make_async_copy(stage.at[i], stage.at[i], sems.at[1 + i]).wait()
        lhs = xn[:, 0:npre, :].reshape(rows_pre, dm).astype(BF16)
        for j in range(hc // 2):
            start = i * (dm * hc // 2) + j
            even = stage2d[pl.ds(start, dm // 2, stride=hc), :]
            odd = stage2d[pl.ds(start + hc // 2, dm // 2, stride=hc), :]
            pair = ((even & jnp.uint32(0xFFFF)) | (odd << 16),
                    (even >> 16) | (odd & jnp.uint32(0xFFFF0000)))
            for t in range(2):
                slot = i * hc + 2 * j + t
                wqkv[slot] = pair[t]
                pre[slot] = pltpu.bitcast(_dot(lhs, pltpu.bitcast(pair[t], BF16)), U32)
        return carry

    lax.fori_loop(0, 3 * nchunk, prologue, 0)

    wo_cp.wait()

    def relay_wo(i, carry):
        wo[pl.ds(i * 256, 256), :] = pltpu.bitcast(wo_raw[pl.ds(i * 512, 512), :], U32)
        return carry

    lax.fori_loop(0, nheads * dh // 512, relay_wo, 0)

    nkeys = nmem + seg + 8
    row = lax.broadcasted_iota(jnp.int32, (seg, nkeys), 0)
    col = lax.broadcasted_iota(jnp.int32, (seg, nkeys), 1)
    real = col < nmem + seg
    mask = real & ((row < nmem) | (col <= row + npre))
    fill = jnp.where(real, _MASKED, -jnp.inf).astype(F32)
    grp = 4
    ngrp = nheads // grp

    def step(s, mem):
        lhs = jnp.concatenate([mem, xn[s, npre:, :]], axis=0).astype(BF16)
        rows = pl.ds(pl.multiple_of(s * npre, npre), npre)
        zeros = jnp.zeros((8, dh), F32)

        def keys(slot):
            p = _dot(lhs, pltpu.bitcast(wqkv[slot], BF16))
            head = jnp.concatenate(
                [p[:nmem], pltpu.bitcast(pre[slot, rows, :], F32)], axis=0).astype(BF16)
            pre[slot, rows, :] = pltpu.bitcast(head, U32)
            tail = jnp.concatenate([p[nmem:], zeros], axis=0).astype(BF16)
            return jnp.concatenate([head, tail], axis=0)

        q, k, v, e, inv, o = {}, {}, {}, {}, {}, {}

        def project(g):
            for h in range(g * grp, (g + 1) * grp):
                q[h] = _dot(lhs, pltpu.bitcast(wqkv[h], BF16)).astype(BF16)
                k[h] = keys(nheads + h)
                v[h] = keys(2 * nheads + h)

        def scores(g):
            for h in range(g * grp, (g + 1) * grp):
                e[h], inv[h] = _softmax_terms(_dot_nt(q[h], k[h]), mask, fill, scale)

        def values(g):
            for h in range(g * grp, (g + 1) * grp):
                o[h] = (_dot(e[h], v[h]) * inv[h]).astype(BF16)

        def out_proj(g):
            lhs_o = jnp.concatenate([o[h] for h in range(g * grp, (g + 1) * grp)], axis=1)
            w = wo[pl.ds(g * grp * dh // 2, grp * dh // 2), :]
            return _dot(lhs_o, pltpu.bitcast(w, BF16))

        for g in range(ngrp):
            project(g)
            if g >= 1:
                scores(g - 1)
            if g >= 2:
                values(g - 2)
        acc = out_proj(0) + out_proj(1)
        scores(ngrp - 1)
        values(ngrp - 2)
        acc = acc + out_proj(2) + out_proj(3) + out_proj(4)
        values(ngrp - 1)
        for g in range(5, ngrp):
            acc = acc + out_proj(g)
        att[s, npre:, :] = acc[nmem:]
        return acc[:nmem]

    lax.fori_loop(0, nseg, step, mem0_ref[...].astype(F32))

    eseg = 8
    erow = lax.broadcasted_iota(jnp.int32, (eseg * npre, eseg * (nmem + npre)), 0)
    ecol = lax.broadcasted_iota(jnp.int32, (eseg * npre, eseg * (nmem + npre)), 1)
    same = (erow // npre) == (ecol // (nmem + npre))
    emask = same & ((ecol % (nmem + npre)) <= (erow % npre) + nmem)
    efill = jnp.where(same, _MASKED, -jnp.inf).astype(F32)
    wr = jnp.broadcast_to(wr_ref[...], (16, dm))

    def attend_pre(g):
        rows = pl.ds(pl.multiple_of(g * eseg * npre, eseg * npre), eseg * npre)
        e, inv, o = {}, {}, {}

        def scores(c):
            for h in range(c * grp, (c + 1) * grp):
                q = pltpu.bitcast(pre[h, rows, :], F32).astype(BF16)
                k = pltpu.bitcast(pre[nheads + h, rows, :], BF16)
                e[h], inv[h] = _softmax_terms(_dot_nt(q, k), emask, efill, scale)

        def values(c):
            for h in range(c * grp, (c + 1) * grp):
                v = pltpu.bitcast(pre[2 * nheads + h, rows, :], BF16)
                o[h] = (_dot(e[h], v) * inv[h]).astype(BF16)

        def out_proj(c):
            lhs_o = jnp.concatenate([o[h] for h in range(c * grp, (c + 1) * grp)], axis=1)
            w = wo[pl.ds(c * grp * dh // 2, grp * dh // 2), :]
            return _dot(lhs_o, pltpu.bitcast(w, BF16))

        acc = None
        for c in range(ngrp + 3):
            if c < ngrp:
                scores(c)
            if 2 <= c < ngrp + 2:
                values(c - 2)
            if c >= 3:
                acc = out_proj(c - 3) if acc is None else acc + out_proj(c - 3)
        att[pl.ds(g * eseg, eseg), 0:npre, :] = acc.reshape(eseg, npre, dm)

    def finish(g):
        segs = pl.ds(g * eseg, eseg)
        a = att[segs].reshape(eseg * seg, dm)
        h = _rnd(x_v[segs].astype(F32).reshape(eseg * seg, dm) + _rnd(a))
        hn = _layernorm(h)
        att[segs] = h.reshape(eseg, seg, dm)
        xn[segs] = hn.reshape(eseg, seg, dm)
        out_v[segs] = (h + hn).astype(BF16).reshape(eseg, seg, dm)
        r_v[g] = _dot_nt(wr, hn.astype(BF16))[:8]

    attend_pre(0)

    def epilogue(g, carry):
        finish(g - 1)
        attend_pre(g)
        return carry

    lax.fori_loop(1, nseg // eseg, epilogue, 0)
    finish(nseg // eseg - 1)

    ntok = nseg * seg
    sub = lax.broadcasted_iota(jnp.int32, (nseg // eseg, eseg * seg), 0)
    tok = sub * (eseg * seg) + lax.broadcasted_iota(jnp.int32, (nseg // eseg, eseg * seg), 1)
    r = r_v[0]
    for g in range(1, nseg // eseg):
        r = jnp.where(sub == g, r_v[g], r)
    r = _rnd(r)
    r = jnp.where(r != r, -jnp.inf, r)
    picked, gates = [], []
    free = tok >= 0
    for _ in range(_TOPC):
        best = jnp.max(jnp.where(free, r, -jnp.inf), keepdims=True)
        idx = jnp.min(jnp.where(free & (r == best), tok, ntok - 1), keepdims=True)
        free = free & (tok != idx)
        picked.append(idx[0, 0])
        gates.append(best)

    r16 = lax.broadcasted_iota(jnp.int32, (16, dm), 0)
    h_sel = jnp.zeros((16, dm), F32)
    hn_sel = jnp.zeros((16, dm), F32)
    gate = jnp.zeros((16, dm), F32)
    for c, idx in enumerate(picked):
        at = (idx // seg, pl.ds(idx % seg, 1), slice(None))
        h_sel = jnp.where(r16 == c, att[at], h_sel)
        hn_sel = jnp.where(r16 == c, xn[at], hn_sel)
        gate = jnp.where(r16 == c, gates[c], gate)

    for cp in ffn_cps:
        cp.wait()
    sel = hn_sel.astype(BF16)
    a = _rnd(_dot(sel, wg_v[...]))
    u = _rnd(_dot(sel, wu_v[...]))
    g_act = _rnd(a * _rnd(jax.nn.sigmoid(a)))
    y = _rnd(_dot((g_act * u).astype(BF16), wd_v[...]))
    y = _rnd(y * _rnd(jax.nn.sigmoid(gate)))
    new = h_sel + _rnd(hn_sel + y)

    rseg = lax.broadcasted_iota(jnp.int32, (seg, dm), 0)
    for c, idx in enumerate(picked):
        old = out_v[idx // seg].astype(F32)
        out_v[idx // seg] = jnp.where(rseg == idx % seg, new[c:c + 1], old).astype(BF16)

    out_cp = pltpu.make_async_copy(out_v, out_hbm, sems.at[0])
    out_cp.start()
    out_cp.wait()


@functools.partial(jax.jit, static_argnames=("A_seg_len",))
def pallas_sequential_preLN__memory_aug_recurrent_mem_tr__moe_arch_mod__prompt_kernel(
    A_x, A_mem0, A_Wq, A_Wk, A_Wv, A_Wo, A_seg_len, B_x, B_w_r, B_w_gate, B_w_up, B_w_down,
):
    del B_x
    batch, ntok, dm = A_x.shape
    _, nheads, dh = A_Wq.shape
    nmem = A_mem0.shape[1]
    seg = int(A_seg_len)
    nseg = ntok // seg
    dff = B_w_gate.shape[1]
    assert (batch, nmem, seg, dh) == (1, 8, 32, 128) and ntok == nseg * seg
    assert nseg == 64 and nheads == 32

    hbm = pl.BlockSpec(memory_space=pl.ANY)
    vmem = pl.BlockSpec(memory_space=pltpu.VMEM)
    out = pl.pallas_call(
        functools.partial(_kernel, nseg=nseg, seg=seg, nmem=nmem, nheads=nheads, dh=dh, dm=dm),
        out_shape=jax.ShapeDtypeStruct((nseg, seg, dm), A_x.dtype),
        in_specs=[hbm, vmem, hbm, hbm, hbm, hbm, vmem, hbm, hbm, hbm],
        out_specs=hbm,
        scratch_shapes=[
            pltpu.VMEM((nseg, seg, dm), BF16),
            pltpu.VMEM((3 * nheads // 16, dm, 8, dh), U32),
            pltpu.VMEM((nheads * dh, dm), BF16),
            pltpu.VMEM((dm, dff), BF16),
            pltpu.VMEM((dm, dff), BF16),
            pltpu.VMEM((dff, dm), BF16),
            pltpu.VMEM((3 * nheads, dm // 2, dh), U32),
            pltpu.VMEM((nheads * dh // 2, dm), U32),
            pltpu.VMEM((nseg, seg, dm), F32),
            pltpu.VMEM((3 * nheads, nseg * nmem, dh), U32),
            pltpu.VMEM((nseg, seg, dm), F32),
            pltpu.VMEM((nseg // 8, 8, 8 * seg), F32),
            pltpu.VMEM((nseg, seg, dm), BF16),
            pltpu.SemaphoreType.DMA((16,)),
        ],
        compiler_params=pltpu.CompilerParams(vmem_limit_bytes=110 * 1024 * 1024),
        name="rmt_mod_block",
    )(
        A_x.reshape(nseg, seg, dm), A_mem0.reshape(nmem, dm), A_Wq, A_Wk, A_Wv,
        A_Wo.reshape(nheads * dh, dm), B_w_r.reshape(1, dm), B_w_gate, B_w_up, B_w_down,
    )
    return out.reshape(batch, ntok, dm)
```

```python
import functools

import jax
import jax.numpy as jnp
import numpy as np
from jax import lax
from jax.experimental import pallas as pl
from jax.experimental.pallas import tpu as pltpu

F32 = jnp.float32
BF16 = jnp.bfloat16
U32 = jnp.uint32

_EPS = float(np.asarray(1e-5, dtype=BF16))
_LOG2E = float(np.log2(np.e))
_MASKED = -1000000000.0
_NT = (((1,), (1,)), ((), ()))
_TOPC = 2
_BLK = 4


def _rnd(a):
    return a.astype(BF16).astype(F32)


def _layernorm(a):
    n = a.shape[-1]
    mean = jnp.sum(a, axis=-1, keepdims=True) * (1.0 / n)
    cen = a - mean
    var = jnp.sum(cen * cen, axis=-1, keepdims=True) * (1.0 / n)
    std = _rnd(jnp.sqrt(_rnd(_rnd(var) + _EPS)))
    return _rnd(_rnd(a - _rnd(mean)) * (1.0 / std))


def _dot(a, b):
    return jnp.dot(a, b, preferred_element_type=F32)


def _dot_nt(a, b):
    return lax.dot_general(a, b, _NT, preferred_element_type=F32)


def _softmax(scores, mask, fill, scale):
    s = jnp.where(mask, scores, fill)
    e = jnp.exp2((s - jnp.max(s, axis=-1, keepdims=True)) * (scale * _LOG2E))
    total = jnp.sum(e, axis=-1, keepdims=True)
    inv = pl.reciprocal(total, approx=True)
    inv = inv * (2.0 - total * inv)
    return (e * inv).astype(BF16)


def _kernel(x_hbm, mem0_ref, wq_hbm, wk_hbm, wv_hbm, wo_hbm, wr_ref, wg_hbm, wu_hbm, wd_hbm,
            out_hbm,
            x_pre, x_v, stage, wo_raw, wg_v, wu_v, wd_v, wqkv, wo, lhs_pre, xn, pre, kv_cur, kv_old, o, o_def,
            att, h_v, hn_v, r_v, out_v, sems, out_sems,
            *, nseg, seg, nmem, nheads, dh, dm):
    scale = float(np.asarray(dh ** -0.5, dtype=BF16))
    npre = nmem
    hc = 16
    nchunk = 3 * nheads // hc
    blk = _BLK
    nblk = nseg // blk
    grp = 4
    ngrp = nheads // grp

    xp_cp = pltpu.make_async_copy(x_hbm.at[:, pl.ds(0, npre), :], x_pre, sems.at[nchunk])
    xp_cp.start()
    for m, w_hbm in enumerate((wq_hbm, wk_hbm, wv_hbm)):
        w32 = w_hbm.bitcast(U32)
        for c in range(nheads // hc):
            i = m * (nheads // hc) + c
            pltpu.make_async_copy(
                w32.at[:, pl.ds(c * hc // 2, hc // 2), :], stage.at[i], sems.at[i]).start()
    late = [pltpu.make_async_copy(src, dst, sems.at[nchunk + 1 + i])
            for i, (src, dst) in enumerate(((wo_hbm, wo_raw), (x_hbm, x_v), (wg_hbm, wg_v),
                                            (wu_hbm, wu_v), (wd_hbm, wd_v)))]
    for cp in late:
        cp.start()

    xp_cp.wait()

    def ln_pre(g, carry):
        a = x_pre[pl.ds(g * 32, 32)].astype(F32).reshape(32 * npre, dm)
        lhs_pre[pl.ds(g * 32 * npre, 32 * npre), :] = _layernorm(a).astype(BF16)
        return carry

    lax.fori_loop(0, nseg // 32, ln_pre, 0)
    att[0:blk, 0:npre, :] = jnp.zeros((blk, npre, dm), F32)
    r_v[...] = jnp.full(r_v.shape, -jnp.inf, F32)

    stage2d = stage.reshape(nchunk * dm * hc // 2, dh)

    def prologue(i, carry):
        pltpu.make_async_copy(stage.at[i], stage.at[i], sems.at[i]).wait()
        for j in range(hc // 2):
            start = i * (dm * hc // 2) + j
            even = stage2d[pl.ds(start, dm // 2, stride=hc), :]
            odd = stage2d[pl.ds(start + hc // 2, dm // 2, stride=hc), :]
            pair = ((even & jnp.uint32(0xFFFF)) | (odd << 16),
                    (even >> 16) | (odd & jnp.uint32(0xFFFF0000)))
            for t in range(2):
                slot = i * hc + 2 * j + t
                wqkv[slot] = pair[t]
                proj = _dot(lhs_pre[...], pltpu.bitcast(pair[t], BF16))
                pre[slot] = pltpu.bitcast(proj.astype(BF16), U32)
        return carry

    lax.fori_loop(0, nchunk, prologue, 0)

    late[0].wait()

    def relay_wo(i, carry):
        wo[pl.ds(i * 256, 256), :] = pltpu.bitcast(wo_raw[pl.ds(i * 512, 512), :], U32)
        return carry

    lax.fori_loop(0, nheads * dh // 512, relay_wo, 0)
    late[1].wait()

    def step_mask(parity):
        row = lax.broadcasted_iota(jnp.int32, (seg, seg + 2 * npre), 0)
        col = lax.broadcasted_iota(jnp.int32, (seg, seg + 2 * npre), 1)
        real = (col < seg) | ((col - seg) // npre == parity)
        mask = real & ((row < nmem) | (col <= row) | (col >= seg))
        return mask, jnp.where(real, _MASKED / scale, -jnp.inf).astype(F32)

    erow = lax.broadcasted_iota(jnp.int32, (blk * npre, 2 * blk * npre), 0)
    ecol = lax.broadcasted_iota(jnp.int32, (blk * npre, 2 * blk * npre), 1)
    same = (erow // npre) == ((ecol // npre) % blk)
    emask = same & (ecol - blk * npre <= erow)
    efill = jnp.where(same, _MASKED / scale, -jnp.inf).astype(F32)

    def put_head(o, h, value):
        o[:, h * dh:(h + 1) * dh] = pltpu.bitcast(value.astype(BF16), U32)

    def out_proj(o, g):
        lhs_o = pltpu.bitcast(o[:, g * grp * dh:(g + 1) * grp * dh], BF16)
        w = wo[pl.ds(g * grp * dh // 2, grp * dh // 2), :]
        return _dot(lhs_o, pltpu.bitcast(w, BF16))

    def norm_in(s):
        xn[...] = _layernorm(x_v[s].astype(F32)[npre:])

    def finish(s):
        h = _rnd(x_v[s].astype(F32) + _rnd(att[s]))
        hn = _layernorm(h)
        h_v[s] = h
        hn_v[s] = hn
        out_v[s] = (h + hn).astype(BF16)
        r = jnp.sum(hn * wr_ref[...].astype(F32), axis=-1, keepdims=True)
        lane = lax.broadcasted_iota(jnp.int32, r_v.shape, 1)
        r_v[...] = jnp.where(lane == s, r, r_v[...])

    class Deferred:
        def __init__(self, b):
            self.b = b
            words = blk * npre // 2
            self.rows = pl.ds(pl.multiple_of(b * words, words), words)
            self.p, self.acc = {}, None
            for h in range(nheads):
                for slot in (h, nheads + h):
                    kv_old[slot] = pltpu.bitcast(kv_cur[slot].astype(BF16), U32)

        def keys(self, slot):
            both = jnp.concatenate([kv_old[slot], pre[nheads + slot, self.rows, :]], axis=0)
            return pltpu.bitcast(both, BF16)

        def scores(self, g):
            for h in range(g * grp, (g + 1) * grp):
                q = pltpu.bitcast(pre[h, self.rows, :], BF16)
                self.p[h] = _softmax(_dot_nt(q, self.keys(h)), emask, efill, scale)

        def values(self, g):
            for h in range(g * grp, (g + 1) * grp):
                put_head(o_def, h, _dot(self.p[h], self.keys(nheads + h)))

        def project(self, g):
            p = out_proj(o_def, g)
            self.acc = p if self.acc is None else self.acc + p

        def store(self):
            att[pl.ds(self.b * blk, blk), 0:npre, :] = self.acc.reshape(blk, npre, dm)

    def step(s, j, mem, side_work, deferred=None, groups=()):
        lhs = jnp.concatenate([mem, xn[...]], axis=0).astype(BF16)
        rows = pl.ds(pl.multiple_of((s // 2) * npre, npre), npre)
        mask, fill = step_mask(j % 2)

        def keys(slot):
            new = _dot(lhs, pltpu.bitcast(wqkv[slot], BF16))
            kv_cur[slot - nheads, pl.ds(j * nmem, nmem), :] = new[:nmem]
            both = [pltpu.bitcast(new.astype(BF16), U32), pre[slot, rows, :]]
            return pltpu.bitcast(jnp.concatenate(both, axis=0), BF16)

        q, k, v, p = {}, {}, {}, {}

        def project(g):
            for h in range(g * grp, (g + 1) * grp):
                q[h] = _dot(lhs, pltpu.bitcast(wqkv[h], BF16)).astype(BF16)
                k[h] = keys(nheads + h)
                v[h] = keys(2 * nheads + h)

        def scores(g):
            for h in range(g * grp, (g + 1) * grp):
                p[h] = _softmax(_dot_nt(q[h], k[h]), mask, fill, scale)

        def values(g):
            for h in range(g * grp, (g + 1) * grp):
                put_head(o, h, _dot(p[h], v[h]))

        for g in range(ngrp):
            project(g)
            if g >= 1:
                scores(g - 1)
            if g >= 2:
                values(g - 2)
            if g < len(groups):
                deferred.scores(groups[g])
            if 2 <= g < len(groups) + 2:
                deferred.values(groups[g - 2])
            if g == 3:
                side_work()
        acc = out_proj(o, 0)
        scores(ngrp - 1)
        acc = acc + out_proj(o, 1) + out_proj(o, 2)
        values(ngrp - 2)
        acc = acc + out_proj(o, 3) + out_proj(o, 4)
        values(ngrp - 1)
        for g in range(5, ngrp):
            acc = acc + out_proj(o, g)
        for g in groups:
            deferred.project(g)
        att[s, npre:, :] = acc[nmem:]
        return acc[:nmem]

    def out_copy(b):
        segs = pl.ds(b * blk, blk)
        return pltpu.make_async_copy(out_v.at[segs], out_hbm.at[segs], out_sems.at[b])

    norm_in(0)

    def first_block(s, mem):
        return step(s, s, mem, lambda: norm_in(s + 1))

    mem = lax.fori_loop(0, blk, first_block, mem0_ref[...].astype(F32))

    def block(b, mem):
        deferred = Deferred(b - 1)
        per = ngrp // blk
        for j in range(blk):
            s = b * blk + j

            def side_work(s=s, j=j):
                norm_in(jnp.minimum(s + 1, nseg - 1))
                finish(jnp.maximum(b - 2, 0) * blk + j)

            mem = step(s, j, mem, side_work, deferred, tuple(range(j * per, (j + 1) * per)))
        deferred.store()

        @pl.when(b >= 2)
        def _():
            out_copy(b - 2).start()

        return mem

    lax.fori_loop(1, nblk, block, mem)

    deferred = Deferred(nblk - 1)
    for g in range(ngrp + 3):
        if g < ngrp:
            deferred.scores(g)
        if 2 <= g < ngrp + 2:
            deferred.values(g - 2)
        if g >= 3:
            deferred.project(g - 3)
    for s in range((nblk - 2) * blk, (nblk - 1) * blk):
        finish(s)
    deferred.store()
    out_copy(nblk - 2).start()
    for s in range((nblk - 1) * blk, nseg):
        finish(s)
    out_copy(nblk - 1).start()

    ntok = nseg * seg
    lane = lax.broadcasted_iota(jnp.int32, r_v.shape, 1)
    tok = lane * seg + lax.broadcasted_iota(jnp.int32, r_v.shape, 0)
    r = _rnd(r_v[...])
    r = jnp.where(r != r, -jnp.inf, r)
    picked, gates = [], []
    free = lane < nseg
    for _ in range(_TOPC):
        best = jnp.max(jnp.where(free, r, -jnp.inf), keepdims=True)
        idx = jnp.min(jnp.where(free & (r == best), tok, ntok - 1), keepdims=True)
        free = free & (tok != idx)
        picked.append(idx[0, 0])
        gates.append(best)

    r16 = lax.broadcasted_iota(jnp.int32, (16, dm), 0)
    h_sel = jnp.zeros((16, dm), F32)
    hn_sel = jnp.zeros((16, dm), F32)
    gate = jnp.zeros((16, dm), F32)
    for c, idx in enumerate(picked):
        at = (idx // seg, pl.ds(idx % seg, 1), slice(None))
        h_sel = jnp.where(r16 == c, h_v[at], h_sel)
        hn_sel = jnp.where(r16 == c, hn_v[at], hn_sel)
        gate = jnp.where(r16 == c, gates[c], gate)

    for cp in late[2:]:
        cp.wait()
    sel = hn_sel.astype(BF16)
    a = _rnd(_dot(sel, wg_v[...]))
    u = _rnd(_dot(sel, wu_v[...]))
    g_act = _rnd(a * _rnd(jax.nn.sigmoid(a)))
    y = _rnd(_dot((g_act * u).astype(BF16), wd_v[...]))
    y = _rnd(y * _rnd(jax.nn.sigmoid(gate)))
    new = h_sel + _rnd(hn_sel + y)

    for b in range(nblk):
        out_copy(b).wait()
    rseg = lax.broadcasted_iota(jnp.int32, (seg, dm), 0)
    for c, idx in enumerate(picked):
        old = out_v[idx // seg].astype(F32)
        out_v[idx // seg] = jnp.where(rseg == idx % seg, new[c:c + 1], old).astype(BF16)

    def fix_copy(c):
        s = pl.ds(picked[c] // seg, 1)
        return pltpu.make_async_copy(out_v.at[s], out_hbm.at[s], out_sems.at[c])

    fix_copy(0).start()

    @pl.when(picked[1] // seg != picked[0] // seg)
    def _():
        fix_copy(1).start()
        fix_copy(1).wait()

    fix_copy(0).wait()


@functools.partial(jax.jit, static_argnames=("A_seg_len",))
def pallas_sequential_preLN__memory_aug_recurrent_mem_tr__moe_arch_mod__prompt_kernel(
    A_x, A_mem0, A_Wq, A_Wk, A_Wv, A_Wo, A_seg_len, B_x, B_w_r, B_w_gate, B_w_up, B_w_down,
):
    del B_x
    batch, ntok, dm = A_x.shape
    _, nheads, dh = A_Wq.shape
    nmem = A_mem0.shape[1]
    seg = int(A_seg_len)
    nseg = ntok // seg
    dff = B_w_gate.shape[1]
    assert (batch, nmem, seg, dh) == (1, 8, 32, 128) and ntok == nseg * seg
    assert nseg == 64 and nheads == 32

    hbm = pl.BlockSpec(memory_space=pl.ANY)
    vmem = pl.BlockSpec(memory_space=pltpu.VMEM)
    out = pl.pallas_call(
        functools.partial(_kernel, nseg=nseg, seg=seg, nmem=nmem, nheads=nheads, dh=dh, dm=dm),
        out_shape=jax.ShapeDtypeStruct((nseg, seg, dm), A_x.dtype),
        in_specs=[hbm, vmem, hbm, hbm, hbm, hbm, vmem, hbm, hbm, hbm],
        out_specs=hbm,
        scratch_shapes=[
            pltpu.VMEM((nseg, nmem, dm), BF16),
            pltpu.VMEM((nseg, seg, dm), BF16),
            pltpu.VMEM((3 * nheads // 16, dm, 8, dh), U32),
            pltpu.VMEM((nheads * dh, dm), BF16),
            pltpu.VMEM((dm, dff), BF16),
            pltpu.VMEM((dm, dff), BF16),
            pltpu.VMEM((dff, dm), BF16),
            pltpu.VMEM((3 * nheads, dm // 2, dh), U32),
            pltpu.VMEM((nheads * dh // 2, dm), U32),
            pltpu.VMEM((nseg * nmem, dm), BF16),
            pltpu.VMEM((seg - nmem, dm), F32),
            pltpu.VMEM((3 * nheads, nseg * nmem // 2, dh), U32),
            pltpu.VMEM((2 * nheads, _BLK * nmem, dh), F32),
            pltpu.VMEM((2 * nheads, _BLK * nmem // 2, dh), U32),
            pltpu.VMEM((seg // 2, nheads * dh), U32),
            pltpu.VMEM((_BLK * nmem // 2, nheads * dh), U32),
            pltpu.VMEM((nseg, seg, dm), F32),
            pltpu.VMEM((nseg, seg, dm), F32),
            pltpu.VMEM((nseg, seg, dm), F32),
            pltpu.VMEM((seg, 128), F32),
            pltpu.VMEM((nseg, seg, dm), BF16),
            pltpu.SemaphoreType.DMA((12,)),
            pltpu.SemaphoreType.DMA((nseg // _BLK,)),
        ],
        compiler_params=pltpu.CompilerParams(vmem_limit_bytes=110 * 1024 * 1024,
                                             disable_bounds_checks=True),
        name="rmt_mod_block",
    )(
        A_x.reshape(nseg, seg, dm), A_mem0.reshape(nmem, dm), A_Wq, A_Wk, A_Wv,
        A_Wo.reshape(nheads * dh, dm), B_w_r.reshape(1, dm), B_w_gate, B_w_up, B_w_down,
    )
    return out.reshape(batch, ntok, dm)
```

```python
import functools

import jax
import jax.numpy as jnp
import numpy as np
from jax import lax
from jax.experimental import pallas as pl
from jax.experimental.pallas import tpu as pltpu

F32 = jnp.float32
BF16 = jnp.bfloat16
U32 = jnp.uint32

_EPS = float(np.asarray(1e-5, dtype=BF16))
_LOG2E = float(np.log2(np.e))
_MASKED = -1000000000.0
_TOPC = 2
_BLK = 4
_GRP = 4
_CHUNK = 16
_PAD = 2


def _rnd(a):
    return a.astype(BF16).astype(F32)


def _layernorm(a):
    n = a.shape[-1]
    mean = jnp.sum(a, axis=-1, keepdims=True) * (1.0 / n)
    cen = a - mean
    var = jnp.sum(cen * cen, axis=-1, keepdims=True) * (1.0 / n)
    std = _rnd(jnp.sqrt(_rnd(_rnd(var) + _EPS)))
    return _rnd(_rnd(a - _rnd(mean)) * (1.0 / std))


def _dot(a, b):
    return jnp.dot(a, b, preferred_element_type=F32)


def _dot_nt(a, b):
    return lax.dot_general(a, b, (((1,), (1,)), ((), ())), preferred_element_type=F32)


def _words(a):
    return pltpu.bitcast(a.astype(BF16), U32)


def _rows(a):
    return pltpu.bitcast(a, BF16)


def _softmax(scores, mask, fill, scale):
    s = jnp.where(mask, scores, fill)
    e = jnp.exp2((s - jnp.max(s, axis=-1, keepdims=True)) * (scale * _LOG2E))
    total = jnp.sum(e, axis=-1, keepdims=True)
    inv = pl.reciprocal(total, approx=True)
    inv = inv * (2.0 - total * inv)
    return (e * inv).astype(BF16)


def _reduce_all(op, a):
    return op(op(a, axis=0, keepdims=True), axis=1, keepdims=True)


def _kernel(x_hbm, mem0_hbm, wq_hbm, wk_hbm, wv_hbm, wo_hbm, wr_hbm, wg_hbm, wu_hbm, wd_hbm,
            out_hbm,
            x_pre, x_v, mem0, wr, stage, wg, wu, wd, wqkv, wo, lhs_pre, xn, pre, kv_cur, kv_old,
            qkv, o_step, o_def, att, h_v, hn_v, out_v, in_sems, out_sems,
            *, nseg, seg, nmem, nheads, dh, dm):
    scale = float(np.asarray(dh ** -0.5, dtype=BF16))
    npre = nmem
    nchunk = 3 * nheads // _CHUNK
    nblk = nseg // _BLK
    ngrp = nheads // _GRP

    def staged(i):
        return stage.at[i, pl.ds(0, dm)]

    x_pre_copy = pltpu.make_async_copy(x_hbm.at[:, pl.ds(0, npre), :], x_pre, in_sems.at[nchunk])
    x_pre_copy.start()
    for m, w_hbm in enumerate((wq_hbm, wk_hbm, wv_hbm)):
        w32 = w_hbm.bitcast(U32)
        for c in range(nheads // _CHUNK):
            i = m * (nheads // _CHUNK) + c
            pltpu.make_async_copy(w32.at[:, pl.ds(c * _CHUNK // 2, _CHUNK // 2), :],
                                  staged(i), in_sems.at[i]).start()
    copies = [pltpu.make_async_copy(src, dst, in_sems.at[nchunk + 1 + i])
              for i, (src, dst) in enumerate((
                  (wo_hbm.bitcast(U32), wo), (x_hbm, x_v), (mem0_hbm, mem0), (wr_hbm, wr),
                  (wg_hbm, wg), (wu_hbm, wu), (wd_hbm, wd)))]
    for copy in copies:
        copy.start()
    loop_copies, ffn_copies = copies[:4], copies[4:]

    x_pre_copy.wait()

    def norm_pre(g, carry):
        a = x_pre[pl.ds(g * 32, 32)].astype(F32).reshape(32 * npre, dm)
        lhs_pre[pl.ds(g * 32 * npre, 32 * npre), :] = _layernorm(a).astype(BF16)
        return carry

    lax.fori_loop(0, nseg // 32, norm_pre, 0)
    att[0:_BLK, 0:npre, :] = jnp.zeros((_BLK, npre, dm), F32)

    scores_at = (3 * nheads, pl.ds(0, seg), slice(None))
    pre[scores_at] = pltpu.bitcast(jnp.full((seg, dh), -jnp.inf, F32), U32)

    stage2d = stage.reshape(nchunk * (dm + _PAD) * _CHUNK // 2, dh)

    def project_pre(i, carry):
        pltpu.make_async_copy(staged(i), staged(i), in_sems.at[i]).wait()
        for j in range(_CHUNK // 2):
            start = i * ((dm + _PAD) * _CHUNK // 2) + j
            even = stage2d[pl.ds(start, dm // 2, stride=_CHUNK), :]
            odd = stage2d[pl.ds(start + _CHUNK // 2, dm // 2, stride=_CHUNK), :]
            pair = ((even & jnp.uint32(0xFFFF)) | (odd << 16),
                    (even >> 16) | (odd & jnp.uint32(0xFFFF0000)))
            for t in range(2):
                slot = i * _CHUNK + 2 * j + t
                wqkv[slot] = pair[t]
                pre[slot] = _words(_dot(lhs_pre[...], _rows(pair[t])))
        return carry

    lax.fori_loop(0, nchunk, project_pre, 0)
    for copy in loop_copies:
        copy.wait()

    def step_mask(parity):
        row = lax.broadcasted_iota(jnp.int32, (seg, seg + 2 * npre), 0)
        col = lax.broadcasted_iota(jnp.int32, (seg, seg + 2 * npre), 1)
        real = (col < seg) | ((col - seg) // npre == parity)
        mask = real & ((row < nmem) | (col <= row) | (col >= seg))
        return mask, jnp.where(real, _MASKED / scale, -jnp.inf).astype(F32)

    drow = lax.broadcasted_iota(jnp.int32, (_BLK * npre, 2 * _BLK * npre), 0)
    dcol = lax.broadcasted_iota(jnp.int32, (_BLK * npre, 2 * _BLK * npre), 1)
    same_segment = (drow // npre) == ((dcol // npre) % _BLK)
    dmask = same_segment & (dcol - _BLK * npre <= drow)
    dfill = jnp.where(same_segment, _MASKED / scale, -jnp.inf).astype(F32)

    def heads(g):
        return range(g * _GRP, (g + 1) * _GRP)

    def put(ref, slot, value):
        ref[:, slot * dh:(slot + 1) * dh] = _words(value)

    def get(ref, slot):
        return ref[:, slot * dh:(slot + 1) * dh]

    def out_proj(o, g):
        width = _GRP * dh
        return _dot(_rows(o[:, g * width:(g + 1) * width]),
                    _rows(wo[pl.ds(g * width // 2, width // 2), :]))

    def norm_in(s):
        xn[...] = _layernorm(x_v[s].astype(F32)[npre:])

    def finish(s):
        h = _rnd(x_v[s].astype(F32) + _rnd(att[s]))
        hn = _layernorm(h)
        h_v[s] = h
        hn_v[s] = hn
        out_v[s] = (h + hn).astype(BF16)
        r = jnp.sum(hn * wr[...].astype(F32).reshape(1, dm), axis=-1, keepdims=True)
        lane = lax.broadcasted_iota(jnp.int32, (seg, dh), 1)
        pre[scores_at] = pltpu.bitcast(
            jnp.where(lane == s, r, pltpu.bitcast(pre[scores_at], F32)), U32)

    class Deferred:
        def __init__(self, b):
            self.b = b
            words = _BLK * npre // 2
            self.rows = pl.ds(pl.multiple_of(b * words, words), words)
            self.p, self.acc = {}, None
            for h in range(nheads):
                for slot in (h, nheads + h):
                    put(kv_old, slot, kv_cur[slot])

        def keys(self, slot):
            return _rows(jnp.concatenate(
                [get(kv_old, slot), pre[nheads + slot, self.rows, :]], axis=0))

        def scores(self, g):
            for h in heads(g):
                q = _rows(pre[h, self.rows, :])
                self.p[h] = _softmax(_dot_nt(q, self.keys(h)), dmask, dfill, scale)

        def values(self, g):
            for h in heads(g):
                put(o_def, h, _dot(self.p[h], self.keys(nheads + h)))

        def project(self, g):
            part = out_proj(o_def, g)
            self.acc = part if self.acc is None else self.acc + part

        def store(self):
            att[pl.ds(self.b * _BLK, _BLK), 0:npre, :] = self.acc.reshape(_BLK, npre, dm)

    def step(s, j, mem, side_work, deferred=None, groups=()):
        lhs = jnp.concatenate([mem, xn[...]], axis=0).astype(BF16)
        rows = pl.ds(pl.multiple_of((s // 2) * npre, npre), npre)
        mask, fill = step_mask(j % 2)
        p = {}

        def keys(slot):
            return _rows(jnp.concatenate([get(qkv, slot), pre[slot, rows, :]], axis=0))

        def project(g):
            for h in heads(g):
                for slot in (h, nheads + h, 2 * nheads + h):
                    new = _dot(lhs, _rows(wqkv[slot]))
                    if slot >= nheads:
                        kv_cur[slot - nheads, pl.ds(j * nmem, nmem), :] = new[:nmem]
                    put(qkv, slot, new)

        def scores(g):
            for h in heads(g):
                p[h] = _softmax(_dot_nt(_rows(get(qkv, h)), keys(nheads + h)), mask, fill, scale)

        def values(g):
            for h in heads(g):
                put(o_step, h, _dot(p[h], keys(2 * nheads + h)))

        for g in range(ngrp):
            project(g)
            if g >= 1:
                scores(g - 1)
            if g >= 2:
                values(g - 2)
            if g < len(groups):
                deferred.scores(groups[g])
            if 2 <= g < len(groups) + 2:
                deferred.values(groups[g - 2])
            if g == 3:
                side_work()
        acc = out_proj(o_step, 0) + out_proj(o_step, 1)
        scores(ngrp - 1)
        acc = acc + out_proj(o_step, 2)
        values(ngrp - 2)
        acc = acc + out_proj(o_step, 3) + out_proj(o_step, 4)
        values(ngrp - 1)
        for g in range(5, ngrp):
            acc = acc + out_proj(o_step, g)
        for g in groups:
            deferred.project(g)
        att[s, npre:, :] = acc[nmem:]
        return acc[:nmem]

    def out_copy(b):
        segs = pl.ds(b * _BLK, _BLK)
        return pltpu.make_async_copy(out_v.at[segs], out_hbm.at[segs], out_sems.at[b])

    norm_in(0)

    def first_block(s, mem):
        return step(s, s, mem, lambda: norm_in(s + 1))

    mem = lax.fori_loop(0, _BLK, first_block, mem0[...].astype(F32))

    def block(b, mem):
        deferred = Deferred(b - 1)
        share = ngrp // _BLK
        for j in range(_BLK):
            s = b * _BLK + j

            def side_work(s=s, j=j):
                norm_in(jnp.minimum(s + 1, nseg - 1))
                finish(jnp.maximum(b - 2, 0) * _BLK + j)

            mem = step(s, j, mem, side_work, deferred, range(j * share, (j + 1) * share))
        deferred.store()

        @pl.when(b >= 2)
        def _():
            out_copy(b - 2).start()

        return mem

    lax.fori_loop(1, nblk, block, mem)

    deferred = Deferred(nblk - 1)
    for g in range(ngrp):
        deferred.scores(g)
    for g in range(ngrp):
        deferred.values(g)
        if g == ngrp - 1:
            for s in range((nblk - 2) * _BLK, (nblk - 1) * _BLK):
                finish(s)
        if g >= 3:
            deferred.project(g - 3)
    for g in range(ngrp - 3, ngrp):
        deferred.project(g)
    deferred.store()
    out_copy(nblk - 2).start()
    for s in range((nblk - 1) * _BLK, nseg):
        finish(s)
    out_copy(nblk - 1).start()

    lane = lax.broadcasted_iota(jnp.int32, (seg, dh), 1)
    token = (lane * seg + lax.broadcasted_iota(jnp.int32, (seg, dh), 0)).astype(F32)
    r = _rnd(pltpu.bitcast(pre[scores_at], F32))
    r = jnp.where(r != r, -jnp.inf, r)
    free = lane < nseg
    picked, gates = [], []
    for _ in range(_TOPC):
        best = _reduce_all(jnp.max, jnp.where(free, r, -jnp.inf))
        first = _reduce_all(jnp.min, jnp.where(free & (r == best), token, nseg * seg - 1.0))
        free = free & (token != first)
        picked.append(first.astype(jnp.int32)[0, 0])
        gates.append(best)

    sel_row = lax.broadcasted_iota(jnp.int32, (16, dm), 0)
    h_sel = jnp.zeros((16, dm), F32)
    hn_sel = jnp.zeros((16, dm), F32)
    gate = jnp.zeros((16, dm), F32)
    for c, idx in enumerate(picked):
        at = (idx // seg, pl.ds(idx % seg, 1), slice(None))
        h_sel = jnp.where(sel_row == c, h_v[at], h_sel)
        hn_sel = jnp.where(sel_row == c, hn_v[at], hn_sel)
        gate = jnp.where(sel_row == c, gates[c], gate)

    for copy in ffn_copies:
        copy.wait()
    sel = hn_sel.astype(BF16)
    a = _rnd(_dot(sel, wg[...]))
    u = _rnd(_dot(sel, wu[...]))
    y = _rnd(_dot((_rnd(a * _rnd(jax.nn.sigmoid(a))) * u).astype(BF16), wd[...]))
    y = _rnd(y * _rnd(jax.nn.sigmoid(gate)))
    routed = h_sel + _rnd(hn_sel + y)

    for b in range(nblk):
        out_copy(b).wait()
    seg_row = lax.broadcasted_iota(jnp.int32, (seg, dm), 0)
    for c, idx in enumerate(picked):
        old = out_v[idx // seg].astype(F32)
        out_v[idx // seg] = jnp.where(seg_row == idx % seg, routed[c:c + 1], old).astype(BF16)

    def patch_copy(c):
        s = pl.ds(picked[c] // seg, 1)
        return pltpu.make_async_copy(out_v.at[s], out_hbm.at[s], out_sems.at[c])

    patch_copy(0).start()

    @pl.when(picked[1] // seg != picked[0] // seg)
    def _():
        patch_copy(1).start()
        patch_copy(1).wait()

    patch_copy(0).wait()


@functools.partial(jax.jit, static_argnames=("A_seg_len",))
def pallas_sequential_preLN__memory_aug_recurrent_mem_tr__moe_arch_mod__prompt_kernel(
    A_x, A_mem0, A_Wq, A_Wk, A_Wv, A_Wo, A_seg_len, B_x, B_w_r, B_w_gate, B_w_up, B_w_down,
):
    del B_x
    batch, ntok, dm = A_x.shape
    _, nheads, dh = A_Wq.shape
    nmem = A_mem0.shape[1]
    seg = int(A_seg_len)
    nseg = ntok // seg
    dff = B_w_gate.shape[1]
    assert (batch, nmem, seg, dh, nheads) == (1, 8, 32, 128, 32)
    assert ntok == nseg * seg and nseg % 32 == 0 and nseg <= dh
    nchunk = 3 * nheads // _CHUNK

    hbm = pl.BlockSpec(memory_space=pl.ANY)
    out = pl.pallas_call(
        functools.partial(_kernel, nseg=nseg, seg=seg, nmem=nmem, nheads=nheads, dh=dh, dm=dm),
        out_shape=jax.ShapeDtypeStruct((nseg, seg, dm), A_x.dtype),
        in_specs=[hbm] * 10,
        out_specs=hbm,
        scratch_shapes=[
            pltpu.VMEM((nseg, nmem, dm), BF16),
            pltpu.VMEM((nseg, seg, dm), BF16),
            pltpu.VMEM((nmem, dm), BF16),
            pltpu.VMEM((dm,), BF16),
            pltpu.VMEM((nchunk, dm + _PAD, _CHUNK // 2, dh), U32),
            pltpu.VMEM((dm, dff), BF16),
            pltpu.VMEM((dm, dff), BF16),
            pltpu.VMEM((dff, dm), BF16),
            pltpu.VMEM((3 * nheads, dm // 2, dh), U32),
            pltpu.VMEM((nheads * dh // 2, dm), U32),
            pltpu.VMEM((nseg * nmem, dm), BF16),
            pltpu.VMEM((seg - nmem, dm), F32),
            pltpu.VMEM((3 * nheads + 1, nseg * nmem // 2, dh), U32),
            pltpu.VMEM((2 * nheads, _BLK * nmem, dh), F32),
            pltpu.VMEM((_BLK * nmem // 2, 2 * nheads * dh), U32),
            pltpu.VMEM((seg // 2, 3 * nheads * dh), U32),
            pltpu.VMEM((seg // 2, nheads * dh), U32),
            pltpu.VMEM((_BLK * nmem // 2, nheads * dh), U32),
            pltpu.VMEM((nseg, seg, dm), F32),
            pltpu.VMEM((nseg, seg, dm), F32),
            pltpu.VMEM((nseg, seg, dm), F32),
            pltpu.VMEM((nseg, seg, dm), BF16),
            pltpu.SemaphoreType.DMA((nchunk + 8,)),
            pltpu.SemaphoreType.DMA((nseg // _BLK,)),
        ],
        compiler_params=pltpu.CompilerParams(
            vmem_limit_bytes=100 * 1024 * 1024, disable_bounds_checks=True),
        name="rmt_mod_block",
    )(
        A_x.reshape(nseg, seg, dm), A_mem0.reshape(nmem, dm), A_Wq, A_Wk, A_Wv,
        A_Wo.reshape(nheads * dh, dm), B_w_r, B_w_gate, B_w_up, B_w_down,
    )
    return out.reshape(batch, ntok, dm)
```

```python
import functools

import jax
import jax.numpy as jnp
import numpy as np
from jax import lax
from jax.experimental import pallas as pl
from jax.experimental.pallas import tpu as pltpu

F32 = jnp.float32
BF16 = jnp.bfloat16
U32 = jnp.uint32

_EPS = float(np.asarray(1e-5, dtype=BF16))
_LOG2E = float(np.log2(np.e))
_MASKED = -1000000000.0
_TOPC = 2
_BLK = 4
_GRP = 4
_CHUNK = 16
_PAD = 2


def _rnd(a):
    return a.astype(BF16).astype(F32)


def _layernorm(a):
    n = a.shape[-1]
    mean = jnp.sum(a, axis=-1, keepdims=True) * (1.0 / n)
    cen = a - mean
    var = jnp.sum(cen * cen, axis=-1, keepdims=True) * (1.0 / n)
    std = _rnd(jnp.sqrt(_rnd(_rnd(var) + _EPS)))
    return _rnd(_rnd(a - _rnd(mean)) * (1.0 / std))


def _sigmoid(a):
    return _rnd(1.0 / _rnd(1.0 + _rnd(jnp.exp(-a))))


def _dot(a, b):
    return jnp.dot(a, b, preferred_element_type=F32)


def _dot_nt(a, b):
    return lax.dot_general(a, b, (((1,), (1,)), ((), ())), preferred_element_type=F32)


def _words(a):
    return pltpu.bitcast(a.astype(BF16), U32)


def _rows(a):
    return pltpu.bitcast(a, BF16)


def _softmax(scores, mask, fill, scale):
    s = jnp.where(mask, scores, fill)
    e = jnp.exp2((s - jnp.max(s, axis=-1, keepdims=True)) * (scale * _LOG2E))
    total = jnp.sum(e, axis=-1, keepdims=True)
    inv = pl.reciprocal(total, approx=True)
    inv = inv * (2.0 - total * inv)
    return (e * inv).astype(BF16)


def _reduce_all(op, a):
    return op(op(a, axis=0, keepdims=True), axis=1, keepdims=True)


def _kernel(x_hbm, mem0_hbm, wq_hbm, wk_hbm, wv_hbm, wo_hbm, wr_hbm, wg_hbm, wu_hbm, wd_hbm,
            out_hbm,
            x_pre, x_v, mem0, wr, stage, wg, wu, wd, wqkv, wo, lhs_pre, xn, pre, kv_cur, kv_old,
            qkv, o_step, o_def, att, h_v, hn_v, out_v, in_sems, out_sems,
            *, nseg, seg, nmem, nheads, dh, dm):
    scale = float(np.asarray(dh ** -0.5, dtype=BF16))
    npre = nmem
    nchunk = 3 * nheads // _CHUNK
    nblk = nseg // _BLK
    ngrp = nheads // _GRP

    def staged(i):
        return stage.at[i, pl.ds(0, dm)]

    x_pre_copy = pltpu.make_async_copy(x_hbm.at[:, pl.ds(0, npre), :], x_pre, in_sems.at[nchunk])
    x_pre_copy.start()
    for m, w_hbm in enumerate((wq_hbm, wk_hbm, wv_hbm)):
        w32 = w_hbm.bitcast(U32)
        for c in range(nheads // _CHUNK):
            i = m * (nheads // _CHUNK) + c
            pltpu.make_async_copy(w32.at[:, pl.ds(c * _CHUNK // 2, _CHUNK // 2), :],
                                  staged(i), in_sems.at[i]).start()
    copies = [pltpu.make_async_copy(src, dst, in_sems.at[nchunk + 1 + i])
              for i, (src, dst) in enumerate((
                  (wo_hbm.bitcast(U32), wo), (x_hbm, x_v), (mem0_hbm, mem0), (wr_hbm, wr),
                  (wg_hbm, wg), (wu_hbm, wu), (wd_hbm, wd)))]
    for copy in copies:
        copy.start()
    loop_copies, ffn_copies = copies[:4], copies[4:]

    x_pre_copy.wait()

    def norm_pre(g, carry):
        a = x_pre[pl.ds(g * 32, 32)].astype(F32).reshape(32 * npre, dm)
        lhs_pre[pl.ds(g * 32 * npre, 32 * npre), :] = _layernorm(a).astype(BF16)
        return carry

    lax.fori_loop(0, nseg // 32, norm_pre, 0)
    att[0:_BLK, 0:npre, :] = jnp.zeros((_BLK, npre, dm), F32)

    scores_at = (3 * nheads, pl.ds(0, seg), slice(None))
    pre[scores_at] = pltpu.bitcast(jnp.full((seg, dh), -jnp.inf, F32), U32)

    stage2d = stage.reshape(nchunk * (dm + _PAD) * _CHUNK // 2, dh)

    def project_pre(i, carry):
        pltpu.make_async_copy(staged(i), staged(i), in_sems.at[i]).wait()
        for j in range(_CHUNK // 2):
            start = i * ((dm + _PAD) * _CHUNK // 2) + j
            even = stage2d[pl.ds(start, dm // 2, stride=_CHUNK), :]
            odd = stage2d[pl.ds(start + _CHUNK // 2, dm // 2, stride=_CHUNK), :]
            pair = ((even & jnp.uint32(0xFFFF)) | (odd << 16),
                    (even >> 16) | (odd & jnp.uint32(0xFFFF0000)))
            for t in range(2):
                slot = i * _CHUNK + 2 * j + t
                wqkv[slot] = pair[t]
                pre[slot] = _words(_dot(lhs_pre[...], _rows(pair[t])))
        return carry

    lax.fori_loop(0, nchunk, project_pre, 0)
    for copy in loop_copies:
        copy.wait()

    def step_mask(parity):
        row = lax.broadcasted_iota(jnp.int32, (seg, seg + 2 * npre), 0)
        col = lax.broadcasted_iota(jnp.int32, (seg, seg + 2 * npre), 1)
        real = (col < seg) | ((col - seg) // npre == parity)
        mask = real & ((row < nmem) | (col <= row) | (col >= seg))
        return mask, jnp.where(real, _MASKED / scale, -jnp.inf).astype(F32)

    drow = lax.broadcasted_iota(jnp.int32, (_BLK * npre, 2 * _BLK * npre), 0)
    dcol = lax.broadcasted_iota(jnp.int32, (_BLK * npre, 2 * _BLK * npre), 1)
    same_segment = (drow // npre) == ((dcol // npre) % _BLK)
    dmask = same_segment & (dcol - _BLK * npre <= drow)
    dfill = jnp.where(same_segment, _MASKED / scale, -jnp.inf).astype(F32)

    def heads(g):
        return range(g * _GRP, (g + 1) * _GRP)

    def put(ref, slot, value):
        ref[:, slot * dh:(slot + 1) * dh] = _words(value)

    def get(ref, slot):
        return ref[:, slot * dh:(slot + 1) * dh]

    def out_proj(o, g):
        width = _GRP * dh
        return _dot(_rows(o[:, g * width:(g + 1) * width]),
                    _rows(wo[pl.ds(g * width // 2, width // 2), :]))

    def norm_in(s):
        xn[...] = _layernorm(x_v[s].astype(F32)[npre:])

    def finish(s):
        h = _rnd(x_v[s].astype(F32) + _rnd(att[s]))
        hn = _layernorm(h)
        h_v[s] = h
        hn_v[s] = hn
        out_v[s] = (h + hn).astype(BF16)
        r = jnp.sum(hn * wr[...].astype(F32).reshape(1, dm), axis=-1, keepdims=True)
        lane = lax.broadcasted_iota(jnp.int32, (seg, dh), 1)
        pre[scores_at] = pltpu.bitcast(
            jnp.where(lane == s, r, pltpu.bitcast(pre[scores_at], F32)), U32)

    class Deferred:
        def __init__(self, b):
            self.b = b
            words = _BLK * npre // 2
            self.rows = pl.ds(pl.multiple_of(b * words, words), words)
            self.p, self.acc = {}, None
            for h in range(nheads):
                for slot in (h, nheads + h):
                    put(kv_old, slot, kv_cur[slot])

        def keys(self, slot):
            return _rows(jnp.concatenate(
                [get(kv_old, slot), pre[nheads + slot, self.rows, :]], axis=0))

        def scores(self, g):
            for h in heads(g):
                q = _rows(pre[h, self.rows, :])
                self.p[h] = _softmax(_dot_nt(q, self.keys(h)), dmask, dfill, scale)

        def values(self, g):
            for h in heads(g):
                put(o_def, h, _dot(self.p[h], self.keys(nheads + h)))

        def project(self, g):
            part = out_proj(o_def, g)
            self.acc = part if self.acc is None else self.acc + part

        def store(self):
            att[pl.ds(self.b * _BLK, _BLK), 0:npre, :] = self.acc.reshape(_BLK, npre, dm)

    def step(s, j, mem, side_work, deferred=None, groups=()):
        lhs = jnp.concatenate([mem, xn[...]], axis=0).astype(BF16)
        rows = pl.ds(pl.multiple_of((s // 2) * npre, npre), npre)
        mask, fill = step_mask(j % 2)
        p = {}

        def keys(slot):
            return _rows(jnp.concatenate([get(qkv, slot), pre[slot, rows, :]], axis=0))

        def project(g):
            for h in heads(g):
                for slot in (h, nheads + h, 2 * nheads + h):
                    new = _dot(lhs, _rows(wqkv[slot]))
                    if slot >= nheads:
                        kv_cur[slot - nheads, pl.ds(j * nmem, nmem), :] = new[:nmem]
                    put(qkv, slot, new)

        def scores(g):
            for h in heads(g):
                p[h] = _softmax(_dot_nt(_rows(get(qkv, h)), keys(nheads + h)), mask, fill, scale)

        def values(g):
            for h in heads(g):
                put(o_step, h, _dot(p[h], keys(2 * nheads + h)))

        for g in range(ngrp):
            project(g)
            if g >= 1:
                scores(g - 1)
            if g >= 2:
                values(g - 2)
            if g < len(groups):
                deferred.scores(groups[g])
            if 2 <= g < len(groups) + 2:
                deferred.values(groups[g - 2])
            if g == 3:
                side_work()
        acc = out_proj(o_step, 0) + out_proj(o_step, 1)
        scores(ngrp - 1)
        acc = acc + out_proj(o_step, 2)
        values(ngrp - 2)
        acc = acc + out_proj(o_step, 3) + out_proj(o_step, 4)
        values(ngrp - 1)
        for g in range(5, ngrp):
            acc = acc + out_proj(o_step, g)
        for g in groups:
            deferred.project(g)
        att[s, npre:, :] = acc[nmem:]
        return acc[:nmem]

    def out_copy(b):
        segs = pl.ds(b * _BLK, _BLK)
        return pltpu.make_async_copy(out_v.at[segs], out_hbm.at[segs], out_sems.at[b])

    norm_in(0)

    def first_block(s, mem):
        return step(s, s, mem, lambda: norm_in(s + 1))

    mem = lax.fori_loop(0, _BLK, first_block, mem0[...].astype(F32))

    def block(b, mem):
        deferred = Deferred(b - 1)
        share = ngrp // _BLK
        for j in range(_BLK):
            s = b * _BLK + j

            def side_work(s=s, j=j):
                norm_in(jnp.minimum(s + 1, nseg - 1))
                finish(jnp.maximum(b - 2, 0) * _BLK + j)

            mem = step(s, j, mem, side_work, deferred, range(j * share, (j + 1) * share))
        deferred.store()

        @pl.when(b >= 2)
        def _():
            out_copy(b - 2).start()

        return mem

    lax.fori_loop(1, nblk, block, mem)

    deferred = Deferred(nblk - 1)
    for g in range(ngrp):
        deferred.scores(g)
    for g in range(ngrp):
        deferred.values(g)
        if g == ngrp - 1:
            for s in range((nblk - 2) * _BLK, (nblk - 1) * _BLK):
                finish(s)
        if g >= 3:
            deferred.project(g - 3)
    for g in range(ngrp - 3, ngrp):
        deferred.project(g)
    deferred.store()
    out_copy(nblk - 2).start()
    for s in range((nblk - 1) * _BLK, nseg):
        finish(s)
    out_copy(nblk - 1).start()

    lane = lax.broadcasted_iota(jnp.int32, (seg, dh), 1)
    token = (lane * seg + lax.broadcasted_iota(jnp.int32, (seg, dh), 0)).astype(F32)
    r = _rnd(pltpu.bitcast(pre[scores_at], F32))
    r = jnp.where(r != r, -jnp.inf, r)
    free = lane < nseg
    picked, gates = [], []
    for _ in range(_TOPC):
        best = _reduce_all(jnp.max, jnp.where(free, r, -jnp.inf))
        first = _reduce_all(jnp.min, jnp.where(free & (r == best), token, nseg * seg - 1.0))
        free = free & (token != first)
        picked.append(first.astype(jnp.int32)[0, 0])
        gates.append(best)

    sel_row = lax.broadcasted_iota(jnp.int32, (16, dm), 0)
    h_sel = jnp.zeros((16, dm), F32)
    hn_sel = jnp.zeros((16, dm), F32)
    gate = jnp.zeros((16, dm), F32)
    for c, idx in enumerate(picked):
        at = (idx // seg, pl.ds(idx % seg, 1), slice(None))
        h_sel = jnp.where(sel_row == c, h_v[at], h_sel)
        hn_sel = jnp.where(sel_row == c, hn_v[at], hn_sel)
        gate = jnp.where(sel_row == c, gates[c], gate)

    for copy in ffn_copies:
        copy.wait()
    sel = hn_sel.astype(BF16)
    a = _rnd(_dot(sel, wg[...]))
    u = _rnd(_dot(sel, wu[...]))
    y = _rnd(_dot((_rnd(a * _sigmoid(a)) * u).astype(BF16), wd[...]))
    y = _rnd(y * _sigmoid(gate))
    routed = h_sel + _rnd(hn_sel + y)

    for b in range(nblk):
        out_copy(b).wait()
    seg_row = lax.broadcasted_iota(jnp.int32, (seg, dm), 0)
    for c, idx in enumerate(picked):
        old = out_v[idx // seg].astype(F32)
        out_v[idx // seg] = jnp.where(seg_row == idx % seg, routed[c:c + 1], old).astype(BF16)

    def patch_copy(c):
        s = pl.ds(picked[c] // seg, 1)
        return pltpu.make_async_copy(out_v.at[s], out_hbm.at[s], out_sems.at[c])

    patch_copy(0).start()

    @pl.when(picked[1] // seg != picked[0] // seg)
    def _():
        patch_copy(1).start()
        patch_copy(1).wait()

    patch_copy(0).wait()


@functools.partial(jax.jit, static_argnames=("A_seg_len",))
def pallas_sequential_preLN__memory_aug_recurrent_mem_tr__moe_arch_mod__prompt_kernel(
    A_x, A_mem0, A_Wq, A_Wk, A_Wv, A_Wo, A_seg_len, B_x, B_w_r, B_w_gate, B_w_up, B_w_down,
):
    del B_x
    batch, ntok, dm = A_x.shape
    _, nheads, dh = A_Wq.shape
    nmem = A_mem0.shape[1]
    seg = int(A_seg_len)
    nseg = ntok // seg
    dff = B_w_gate.shape[1]
    assert (batch, nmem, seg, dh, nheads) == (1, 8, 32, 128, 32)
    assert ntok == nseg * seg and nseg % 32 == 0 and nseg <= dh
    nchunk = 3 * nheads // _CHUNK

    hbm = pl.BlockSpec(memory_space=pl.ANY)
    out = pl.pallas_call(
        functools.partial(_kernel, nseg=nseg, seg=seg, nmem=nmem, nheads=nheads, dh=dh, dm=dm),
        out_shape=jax.ShapeDtypeStruct((nseg, seg, dm), A_x.dtype),
        in_specs=[hbm] * 10,
        out_specs=hbm,
        scratch_shapes=[
            pltpu.VMEM((nseg, nmem, dm), BF16),
            pltpu.VMEM((nseg, seg, dm), BF16),
            pltpu.VMEM((nmem, dm), BF16),
            pltpu.VMEM((dm,), BF16),
            pltpu.VMEM((nchunk, dm + _PAD, _CHUNK // 2, dh), U32),
            pltpu.VMEM((dm, dff), BF16),
            pltpu.VMEM((dm, dff), BF16),
            pltpu.VMEM((dff, dm), BF16),
            pltpu.VMEM((3 * nheads, dm // 2, dh), U32),
            pltpu.VMEM((nheads * dh // 2, dm), U32),
            pltpu.VMEM((nseg * nmem, dm), BF16),
            pltpu.VMEM((seg - nmem, dm), F32),
            pltpu.VMEM((3 * nheads + 1, nseg * nmem // 2, dh), U32),
            pltpu.VMEM((2 * nheads, _BLK * nmem, dh), F32),
            pltpu.VMEM((_BLK * nmem // 2, 2 * nheads * dh), U32),
            pltpu.VMEM((seg // 2, 3 * nheads * dh), U32),
            pltpu.VMEM((seg // 2, nheads * dh), U32),
            pltpu.VMEM((_BLK * nmem // 2, nheads * dh), U32),
            pltpu.VMEM((nseg, seg, dm), F32),
            pltpu.VMEM((nseg, seg, dm), F32),
            pltpu.VMEM((nseg, seg, dm), F32),
            pltpu.VMEM((nseg, seg, dm), BF16),
            pltpu.SemaphoreType.DMA((nchunk + 8,)),
            pltpu.SemaphoreType.DMA((nseg // _BLK,)),
        ],
        compiler_params=pltpu.CompilerParams(vmem_limit_bytes=100 * 1024 * 1024),
        name="rmt_mod_block",
    )(
        A_x.reshape(nseg, seg, dm), A_mem0.reshape(nmem, dm), A_Wq, A_Wk, A_Wv,
        A_Wo.reshape(nheads * dh, dm), B_w_r, B_w_gate, B_w_up, B_w_down,
    )
    return out.reshape(batch, ntok, dm)
```
